```python
import os as _os
_os.environ.setdefault("JAX_PLATFORMS", "cpu")
import jax
import jax.numpy as jnp

def _softmax(x, axis=-1):
    return jax.nn.softmax(x, axis=axis)
def _gelu(x):
    return jax.nn.gelu(x, approximate=True)
def _silu(x):
    return jax.nn.silu(x)
def _sigmoid(x):
    return jax.nn.sigmoid(x)
def _layernorm(x, axis=-1, eps=1e-5):
    m = jnp.mean(x, axis=axis, keepdims=True)
    v = jnp.var(x, axis=axis, keepdims=True)
    return (x - m) / jnp.sqrt(v + eps)
def _scatter_add(tgt, idx, src, axis=0):
    return tgt.at[idx].add(src)
def _segment_sum(src, seg, n):
    return jax.ops.segment_sum(src, seg, n)
class _Rng:
    def __init__(self, key):
        self._k = key
    def _next(self):
        self._k, sub = jax.random.split(self._k)
        return sub
    def normal(self, shape):
        return jax.random.normal(self._next(), shape, dtype=jnp.bfloat16)
    def randint(self, lo, hi, shape):
        return jax.random.randint(self._next(), shape, lo, hi, dtype=jnp.int32)
    def uniform(self, shape, lo=0.0, hi=1.0):
        return jax.random.uniform(self._next(), shape, jnp.bfloat16, lo, hi)
    def permutation(self, n):
        return jax.random.permutation(self._next(), n)


kernel_name = 'sequential_preLN__mha_block__swiglu_ffn__prompt'

def setup_inputs():
    _rng = _Rng(jax.random.key(int.from_bytes(__import__("os").urandom(4), "little")))
    _w = (lambda a: (lambda t: t.astype(jnp.bfloat16) if jnp.issubdtype(t.dtype, jnp.floating) else t)(jnp.asarray(a)))
    def _A_setup():
        B, S, D, H = 1, 2048, 640, 32
        return {
            "x": _w((lambda *s: _rng.normal(s) * 0.05)(B, S, D)),
            "wqkv": _w((lambda *s: _rng.normal(s) * 0.05)(D, 3 * D)),
            "wo": _w((lambda *s: _rng.normal(s) * 0.05)(D, D)),
        }
    _A_in = _A_setup()

    def _B_setup():
        B, S, D, F = 1, 2048, 640, 1728
        return {
            "x": _w((lambda *s: _rng.normal(s) * 0.05)(B, S, D)),
            "w_gate": _w((lambda *s: _rng.normal(s) * 0.05)(D, F)),
            "w_up": _w((lambda *s: _rng.normal(s) * 0.05)(D, F)),
            "w_down": _w((lambda *s: _rng.normal(s) * 0.05)(F, D)),
        }
    _B_in = _B_setup()

    return {
        "A_x": _A_in["x"],
        "A_wqkv": _A_in["wqkv"],
        "A_wo": _A_in["wo"],
        "B_x": _B_in["x"],
        "B_w_gate": _B_in["w_gate"],
        "B_w_up": _B_in["w_up"],
        "B_w_down": _B_in["w_down"],
    }

def reference(A_x, A_wqkv, A_wo, B_x, B_w_gate, B_w_up, B_w_down):
    def _A_ref(x, wqkv, wo):
        B, S, D = x.shape
        H = 32
        Dh = D // H
        qkv = (lambda x, *d: x.transpose(*d))((x @ wqkv).reshape(B, S, 3, H, Dh), 2, 0, 3, 1, 4)
        q, k, v = qkv[0], qkv[1], qkv[2]
        scores = jnp.einsum("bhqd,bhkd->bhqk", q, k) * (Dh ** -0.5)
        p = _softmax(scores, axis=-1)
        o = jnp.einsum("bhqk,bhkd->bhqd", p, v)
        return (lambda x, *d: x.transpose(*d))(o, 0, 2, 1, 3).reshape(B, S, D) @ wo

    def _B_ref(x, w_gate, w_up, w_down):
        g = _silu(x @ w_gate)
        u = x @ w_up
        return (g * u) @ w_down

    x = A_x
    h = x + _A_ref(_layernorm(x, axis=-1), A_wqkv, A_wo)
    h2 = h + _B_ref(_layernorm(h, axis=-1), B_w_gate, B_w_up, B_w_down)
    return h2
```

```python
import math

import jax
import jax.numpy as jnp
from jax import lax
import jax.experimental.pallas as pl
import jax.experimental.pallas.tpu as pltpu

S, D, H, F = 2048, 640, 32, 1728
DH = D // H
TQ = 512
NQ = S // TQ
EPS = 1e-5
QSCALE = (DH ** -0.5) * math.log2(math.e)
KWIN = (0, 112, 240, 352, 480, 512)
L_MIN = 2.0 ** -40
O_MAX = 2.0 ** 70
BF, F32 = jnp.bfloat16, jnp.float32


def _mm(a, b):
    return jnp.dot(a, b, preferred_element_type=F32)


def _ln_t(x):
    xc = x - jnp.mean(x, axis=0, keepdims=True)
    return xc * lax.rsqrt(jnp.mean(xc * xc, axis=0, keepdims=True) + EPS)


def _body(x_hbm, wqkv_hbm, wo_hbm, wgt_hbm, wut_hbm, wd_hbm, out_hbm,
          x_v, wqkv_v, wo_v, wgt_v, wut_v, wd_v, out_v,
          wt_v, wot_v, wdt_v, xt_v, qt_v, k_v, vt_v, ot_v, p_v, sem_x, sem_w, sem_o):
    cp = pltpu.make_async_copy
    chunks = [slice(c * TQ, (c + 1) * TQ) for c in range(NQ)]
    thirds = [slice(j * D, (j + 1) * D) for j in range(3)]
    x_cps = [cp(x_hbm.at[c], x_v.at[c], sem_x.at[i]) for i, c in enumerate(chunks)]
    o_cps = [cp(out_v.at[c], out_hbm.at[c], sem_o.at[i]) for i, c in enumerate(chunks)]
    a_cps = [cp(wqkv_hbm.at[:, c], wqkv_v.at[:, c], sem_w.at[i]) for i, c in enumerate(thirds)]
    b_cps = [cp(s_, d_, sem_w.at[3 + i]) for i, (s_, d_) in enumerate(
        ((wo_hbm, wo_v), (wd_hbm, wd_v), (wgt_hbm, wgt_v), (wut_hbm, wut_v)))]
    for c in [x_cps[0], a_cps[0], a_cps[1], a_cps[2]] + x_cps[1:]:
        c.start()

    def qkv(c, first=False):
        xt = x_v[c, :].astype(F32).T
        xt_v[:, c] = xt
        xn = _ln_t(xt).astype(BF)
        t = []
        for j in range(3):
            if first:
                a_cps[j].wait()
                wt_v[thirds[j], :] = wqkv_v[:, thirds[j]].T
            t.append(_mm(wt_v[thirds[j], :], xn))
        qt_v[:, c] = (t[0] * QSCALE).astype(BF)
        for g, w in enumerate(KWIN):
            k_v[g, c, :] = t[1][w:w + 128].T.astype(BF)
        vt_v[:, c] = t[2].astype(BF)

    x_cps[0].wait()
    qkv(chunks[0], first=True)
    for c in b_cps:
        c.start()
    for c in x_cps[1:]:
        c.wait()
    lax.fori_loop(1, NQ, lambda i, _: qkv(pl.ds(pl.multiple_of(i * TQ, TQ), TQ)), None)

    def scores(h, c):
        g = h // 6
        w0 = pl.multiple_of(jnp.minimum((g * 120) // 16 * 16, 512), 16)
        r = lax.broadcasted_iota(jnp.int32, (128, 128), 0) + (w0 - h * DH)
        msk = jnp.where((r >= 0) & (r < DH), 1.0, 0.0).astype(BF) > 0
        q = qt_v[pl.ds(w0, 128), c]
        q = jnp.concatenate(
            [jnp.where(msk, q[:, j:j + 128], 0) for j in range(0, TQ, 128)], axis=1)
        return _mm(k_v[g], q)

    def weighted(h, c, p, chk):
        w0 = pl.multiple_of((h * DH) // 16 * 16, 16)
        off = h * DH - w0
        r = lax.broadcasted_iota(jnp.int32, (32, 128), 0)
        one = jnp.where(r == jnp.where(off == 0, 31, 0), 1.0, 0.0).astype(BF) > 0
        v = vt_v[pl.ds(w0, 32), :]
        v = jnp.concatenate(
            [jnp.where(one, 1, v[:, j:j + 128]) for j in range(0, S, 128)], axis=1)
        o = _mm(v, p)
        l = jnp.where(off == 0, o[31:32], o[0:1])
        r = lax.broadcasted_iota(jnp.int32, (32, TQ), 0) - off
        pltpu.store(ot_v.at[pl.ds(w0, 32), c], o * (1.0 / l), mask=(r >= 0) & (r < DH))
        a = jnp.abs(o)
        return jnp.minimum(chk[0], l), chk[1] + ((a[0:8] + a[8:16]) + (a[16:24] + a[24:32]))

    def qk_fast(h, i):
        p_v[i % 2] = pltpu.bitcast(jnp.exp2(scores(h, chunks[i])).astype(BF), jnp.uint32)

    def pv_fast(h, i, chk):
        return weighted(h, chunks[i], pltpu.bitcast(p_v[i % 2], BF), chk)

    def head(h, chk, last=False):
        for i in range(NQ):
            if i + 1 < NQ:
                qk_fast(h, i + 1)
            elif not last:
                qk_fast(h + 1, 0)
            chk = pv_fast(h, i, chk)
        return chk

    chk = (jnp.full((1, TQ), 1.0, F32), jnp.zeros((8, TQ), F32))
    qk_fast(0, 0)
    chk = lax.fori_loop(0, H - 1, head, chk)
    for c in b_cps:
        c.wait()
    wot_v[...] = wo_v[...].T
    wdt_v[...] = wd_v[...].T
    chk = head(H - 1, chk, last=True)
    safe = jnp.logical_and(jnp.min(chk[0]) >= L_MIN, jnp.sum(chk[1]) <= O_MAX)

    @pl.when(jnp.logical_not(safe))
    def _():
        def step(t, chk):
            h, c = t // NQ, pl.ds(pl.multiple_of((t % NQ) * TQ, TQ), TQ)
            s = scores(h, c)
            p = jnp.exp2(s - jnp.max(s, axis=0, keepdims=True)).astype(BF)
            return weighted(h, c, p, chk)

        lax.fori_loop(0, H * NQ, step, chk)

    def proj(c):
        h = xt_v[:, c] + _mm(wot_v[...], ot_v[:, c].astype(BF))
        xt_v[:, c] = h
        qt_v[:, c] = _ln_t(h).astype(BF)

    def ffn(c):
        hn = qt_v[:, c]
        g = _mm(wgt_v[...], hn)
        u = _mm(wut_v[...], hn)
        a = (g * jax.nn.sigmoid(g) * u).astype(BF)
        y = xt_v[:, c] + _mm(wdt_v[...], a)
        out_v[c, :] = y.T.astype(BF)

    for c in chunks:
        proj(c)

    def ffn_step(i, _):
        c = pl.ds(pl.multiple_of(i * TQ, TQ), TQ)
        ffn(c)
        cp(out_v.at[c], out_hbm.at[c], sem_o.at[i]).start()

    lax.fori_loop(0, NQ, ffn_step, None)
    for c in o_cps:
        c.wait()


@jax.jit
def pallas_sequential_preLN__mha_block__swiglu_ffn__prompt_kernel(
    A_x: jax.Array,
    A_wqkv: jax.Array,
    A_wo: jax.Array,
    B_x: jax.Array,
    B_w_gate: jax.Array,
    B_w_up: jax.Array,
    B_w_down: jax.Array,
):
    del B_x
    hbm = pl.BlockSpec(memory_space=pltpu.MemorySpace.HBM)
    vm = pltpu.VMEM
    out = pl.pallas_call(
        _body,
        in_specs=[hbm] * 6,
        out_specs=hbm,
        out_shape=jax.ShapeDtypeStruct((S, D), BF),
        scratch_shapes=[
            vm((S, D), BF), vm((D, 3 * D), BF), vm((D, D), BF), vm((F, D), BF),
            vm((F, D), BF), vm((F, D), BF), vm((S, D), BF),
            vm((3 * D, D), BF), vm((D, D), BF), vm((D, F), BF), vm((D, S), F32),
            vm((D, S), BF), vm((6, S, 128), BF), vm((D, S), BF),
            vm((D, S), F32), vm((2, S // 2, TQ), jnp.uint32),
            pltpu.SemaphoreType.DMA((NQ,)), pltpu.SemaphoreType.DMA((7,)),
            pltpu.SemaphoreType.DMA((NQ,)),
        ],
        compiler_params=pltpu.CompilerParams(vmem_limit_bytes=100 * 2 ** 20),
    )(A_x.reshape(S, D), A_wqkv, A_wo, B_w_gate.T, B_w_up.T, B_w_down)
    return out.reshape(1, S, D)
```

```python
import math

import jax
import jax.numpy as jnp
from jax import lax
import jax.experimental.pallas as pl
import jax.experimental.pallas.tpu as pltpu

S, D, H, F = 2048, 640, 32, 1728
DH = D // H
TQ = 512
NQ = S // TQ
EPS = 1e-5
QSCALE = (DH ** -0.5) * math.log2(math.e)
KWIN = (0, 112, 240, 352, 480, 512)
L_MIN = 2.0 ** -40
O_MAX = 2.0 ** 70
HU = 3
ONE2 = 0x3F803F80
BF, F32, I32 = jnp.bfloat16, jnp.float32, jnp.int32


def _pack(x):
    return pltpu.bitcast(x, I32)


def _unpack(x):
    return pltpu.bitcast(x, BF)


def _mm(a, b):
    return jnp.dot(a, b, preferred_element_type=F32)


def _ln_t(x):
    xc = x - jnp.mean(x, axis=0, keepdims=True)
    return xc * lax.rsqrt(jnp.mean(xc * xc, axis=0, keepdims=True) + EPS)


def _body(x_hbm, wqkv_hbm, wo_hbm, wgt_hbm, wut_hbm, wd_hbm, out_hbm,
          x_v, wqkv_v, wo_v, wgt_v, wut_v, wd_v, out_v,
          wt_v, wot_v, wdt_v, xt_v, qt_v, k_v, vt_v, ot_v, p_v, qm_v, o_v, hn_v,
          sem_x, sem_w, sem_o):
    cp = pltpu.make_async_copy
    chunks = [slice(c * TQ, (c + 1) * TQ) for c in range(NQ)]
    thirds = [slice(j * D, (j + 1) * D) for j in range(3)]
    x_cps = [cp(x_hbm.at[c], x_v.at[c], sem_x.at[i]) for i, c in enumerate(chunks)]
    o_cps = [cp(out_v.at[c], out_hbm.at[c], sem_o.at[i]) for i, c in enumerate(chunks)]
    a_cps = [cp(wqkv_hbm.at[:, c], wqkv_v.at[:, c], sem_w.at[i]) for i, c in enumerate(thirds)]
    b_cps = [cp(s_, d_, sem_w.at[3 + i]) for i, (s_, d_) in enumerate(
        ((wo_hbm, wo_v), (wd_hbm, wd_v), (wgt_hbm, wgt_v), (wut_hbm, wut_v)))]
    x_cps[0].start()
    a_cps[0].start()

    def ln1(c):
        xt = x_v[c, :].astype(F32).T
        xt_v[:, c] = xt
        hn_v[:, c] = _ln_t(xt).astype(BF)

    def qkv(c, j):
        t = _mm(wt_v[thirds[j], :], hn_v[:, c])
        if j == 0:
            qt_v[:, c] = _pack((t * QSCALE).astype(BF))
        elif j == 1:
            for g, w in enumerate(KWIN):
                k_v[g, c, :] = t[w:w + 128].T.astype(BF)
        else:
            vt_v[:, c] = _pack(t.astype(BF))

    def wtrans(j):
        wt_v[thirds[j], :] = wqkv_v[:, thirds[j]].T

    x_cps[0].wait()
    a_cps[0].wait()
    a_cps[1].start()
    a_cps[2].start()
    wtrans(0)
    ln1(chunks[0])
    qkv(chunks[0], 0)
    a_cps[1].wait()
    a_cps[2].wait()
    for c in x_cps[1:]:
        c.start()
    for j in (1, 2):
        wtrans(j)
        qkv(chunks[0], j)
    for c in x_cps[1:]:
        c.wait()
    for c in b_cps:
        c.start()
    for c in chunks[1:]:
        ln1(c)
        for j in range(3):
            qkv(c, j)

    def stage_q(h, c):
        g = lax.div(h, 6)
        w0 = pl.multiple_of(jnp.minimum((g * 60) & ~7, 256), 8)
        r = lax.broadcasted_iota(jnp.int32, (64, TQ), 0) + (w0 - h * (DH // 2))
        qm_v[:, c] = jnp.where((r >= 0) & (r < DH // 2), qt_v[pl.ds(w0, 64), c], 0)

    def scores(h, c):
        return _mm(k_v[lax.div(h, 6)], _unpack(qm_v[:, c]))

    def weighted(h, p):
        w0 = pl.multiple_of((h * (DH // 2)) & ~7, 8)
        r = lax.broadcasted_iota(jnp.int32, (16, S), 0)
        one = r == jnp.where(w0 == h * (DH // 2), 15, 0)
        v = jnp.where(one, ONE2, vt_v[pl.ds(w0, 16), :])
        return _mm(_unpack(v), p)

    def finish(h, c, o, chk):
        w0 = pl.multiple_of((h * DH) & ~15, 16)
        off = h * DH - w0
        l = jnp.where(off == 0, o[31:32], o[0:1])
        r = lax.broadcasted_iota(jnp.int32, (32, TQ), 0) - off
        pltpu.store(ot_v.at[pl.ds(w0, 32), c], o * (1.0 / l), mask=(r >= 0) & (r < DH))
        a = jnp.abs(o)
        a = (a[0:8] + a[8:16]) + (a[16:24] + a[24:32])
        a = (a[:, 0:128] + a[:, 128:256]) + (a[:, 256:384] + a[:, 384:512])
        l = jnp.minimum(jnp.minimum(l[:, 0:128], l[:, 128:256]),
                        jnp.minimum(l[:, 256:384], l[:, 384:512]))
        return jnp.minimum(chk[0], l), chk[1] + a

    def qk_fast(h, i):
        p_v[i % 2] = _pack(jnp.exp2(scores(h, chunks[i])).astype(BF))

    def heads(h0, n, chk, last=False):
        steps = [(h0 + dh, i) for dh in range(n + 1) for i in range(NQ)]
        total = n * NQ
        chk = finish(jnp.maximum(h0 - 1, 0), chunks[NQ - 1], o_v[...], chk)
        for t in range(total):
            if not (last and t + 2 >= total):
                stage_q(steps[t + 2][0], chunks[steps[t + 2][1]])
            if not (last and t + 1 >= total):
                qk_fast(*steps[t + 1])
            h, i = steps[t]
            o = weighted(h, _unpack(p_v[i % 2]))
            if t + 1 < total or last:
                chk = finish(h, chunks[i], o, chk)
            else:
                o_v[...] = o
        return chk

    o_v[...] = jnp.ones(o_v.shape, F32)
    stage_q(0, chunks[0])
    stage_q(0, chunks[1])
    qk_fast(0, 0)
    chk = (jnp.ones((1, 128), F32), jnp.zeros((8, 128), F32))
    chk = lax.fori_loop(0, (H - 1) // HU, lambda u, k: heads(u * HU, HU, k), chk)
    for c in b_cps:
        c.wait()
    wot_v[...] = wo_v[...].T
    wdt_v[...] = wd_v[...].T
    h_tail = (H - 1) // HU * HU
    chk = heads(h_tail, H - h_tail, chk, last=True)
    safe = jnp.logical_and(jnp.min(chk[0]) >= L_MIN, jnp.sum(chk[1]) <= O_MAX)

    @pl.when(jnp.logical_not(safe))
    def _():
        def step(t, chk):
            h, c = t // NQ, pl.ds(pl.multiple_of((t % NQ) * TQ, TQ), TQ)
            stage_q(h, c)
            s = scores(h, c)
            p = jnp.exp2(s - jnp.max(s, axis=0, keepdims=True)).astype(BF)
            return finish(h, c, weighted(h, p), chk)

        lax.fori_loop(0, H * NQ, step, chk)

    def proj(c):
        h = xt_v[:, c] + _mm(wot_v[...], ot_v[:, c].astype(BF))
        xt_v[:, c] = h
        hn_v[:, c] = _ln_t(h).astype(BF)

    def ffn(c):
        hn = hn_v[:, c]
        g = _mm(wgt_v[...], hn)
        u = _mm(wut_v[...], hn)
        a = (g * jax.nn.sigmoid(g) * u).astype(BF)
        y = xt_v[:, c] + _mm(wdt_v[...], a)
        out_v[c, :] = y.T.astype(BF)

    def ffn_step(i, _):
        c = pl.ds(pl.multiple_of(i * TQ, TQ), TQ)
        ffn(c)
        cp(out_v.at[c], out_hbm.at[c], sem_o.at[i]).start()

    for c in chunks:
        proj(c)
    lax.fori_loop(0, NQ, ffn_step, None)
    for c in o_cps:
        c.wait()


@jax.jit
def pallas_sequential_preLN__mha_block__swiglu_ffn__prompt_kernel(
    A_x: jax.Array,
    A_wqkv: jax.Array,
    A_wo: jax.Array,
    B_x: jax.Array,
    B_w_gate: jax.Array,
    B_w_up: jax.Array,
    B_w_down: jax.Array,
):
    del B_x
    hbm = pl.BlockSpec(memory_space=pltpu.MemorySpace.HBM)
    vm = pltpu.VMEM
    out = pl.pallas_call(
        _body,
        in_specs=[hbm] * 6,
        out_specs=hbm,
        out_shape=jax.ShapeDtypeStruct((S, D), BF),
        scratch_shapes=[
            vm((S, D), BF), vm((D, 3 * D), BF), vm((D, D), BF), vm((F, D), BF),
            vm((F, D), BF), vm((F, D), BF), vm((S, D), BF),
            vm((3 * D, D), BF), vm((D, D), BF), vm((D, F), BF), vm((D, S), F32),
            vm((D // 2, S), I32), vm((6, S, 128), BF), vm((D // 2, S), I32),
            vm((D, S), F32), vm((2, S // 2, TQ), I32),
            vm((64, S), I32), vm((32, TQ), F32), vm((D, S), BF),
            pltpu.SemaphoreType.DMA((NQ,)), pltpu.SemaphoreType.DMA((7,)),
            pltpu.SemaphoreType.DMA((NQ,)),
        ],
        compiler_params=pltpu.CompilerParams(vmem_limit_bytes=100 * 2 ** 20),
    )(A_x.reshape(S, D), A_wqkv, A_wo, B_w_gate.T, B_w_up.T, B_w_down)
    return out.reshape(1, S, D)
```
